```python
import os as _os
_os.environ.setdefault('JAX_PLATFORMS', 'cpu')
import jax
import jax.numpy as jnp

def _softmax(x, axis=-1):
    return jax.nn.softmax(x, axis=axis)

def _gelu(x):
    return jax.nn.gelu(x, approximate=True)

def _silu(x):
    return jax.nn.silu(x)

def _sigmoid(x):
    return jax.nn.sigmoid(x)

def _layernorm(x, axis=-1, eps=1e-05):
    m = jnp.mean(x, axis=axis, keepdims=True)
    v = jnp.var(x, axis=axis, keepdims=True)
    return (x - m) / jnp.sqrt(v + eps)

def _scatter_add(tgt, idx, src, axis=0):
    return tgt.at[idx].add(src)

def _segment_sum(src, seg, n):
    return jax.ops.segment_sum(src, seg, n)

class _Rng:

    def __init__(self, key):
        self._k = key

    def _next(self):
        self._k, sub = jax.random.split(self._k)
        return sub

    def normal(self, shape):
        return jax.random.normal(self._next(), shape, dtype=jnp.bfloat16)

    def randint(self, lo, hi, shape):
        return jax.random.randint(self._next(), shape, lo, hi, dtype=jnp.int32)

    def uniform(self, shape, lo=0.0, hi=1.0):
        return jax.random.uniform(self._next(), shape, jnp.bfloat16, lo, hi)

    def permutation(self, n):
        return jax.random.permutation(self._next(), n)
kernel_name = 'standalone__conformer_conv_module__speech'

def setup_inputs():
    _rng = _Rng(jax.random.key(int.from_bytes(__import__("os").urandom(4), "little")))
    _w = lambda a: (lambda t: t.astype(jnp.bfloat16) if jnp.issubdtype(t.dtype, jnp.floating) else t)(jnp.asarray(a))
    B, T, D, K = (2, 4000, 512, 15)
    return {'x': _w((lambda *s: _rng.normal(s) * 0.2)(B, T, D)), 'w_pw1': _w((lambda *s: _rng.normal(s) * 0.2)(D, 2 * D)), 'dw': _w((lambda *s: _rng.normal(s) * 0.05)(K, D)), 'w_pw2': _w((lambda *s: _rng.normal(s) * 0.05)(D, D))}

def reference(x, w_pw1, dw, w_pw2):
    B, T, D = x.shape
    K = dw.shape[0]
    h = x @ w_pw1
    a, b = (h[..., :D].copy(), h[..., D:].copy())
    h = a * _sigmoid(b)
    pad = K // 2
    hp = jnp.pad(h, ((0, 0), (pad, pad), (0, 0)))
    out = jnp.zeros_like(h)
    for i in range(K):
        out = out + hp[:, i:i + T, :] * dw[i][None, None, :]
    return _silu(out) @ w_pw2
```

```python
import functools
import jax, jax.numpy as jnp
import numpy as np
from jax import lax
import jax.experimental.pallas as pl
import jax.experimental.pallas.tpu as pltpu

def make(m=80, U=5, RB=80, order=0, flags=None, nbc=False):
    B, T, D, K = 2, 4000, 512, 15
    R = B * T
    M = m * U
    N = R // M
    CG = D // 128
    SH = 8
    NS = 5
    f32, bf16, u32 = jnp.float32, jnp.bfloat16, jnp.uint32

    def kern(x_hbm, w1_hbm, dw_hbm, w2_hbm, o_hbm,
             xb, w1b, w2b, dwb, dwf, stb, sb, ob,
             xsem, wsem, osem):
        cs = lambda c: pl.ds(c * 128, 128)

        def xcopy(i, c):
            return pltpu.make_async_copy(x_hbm.at[pl.ds(i * M, M), cs(c)], xb.at[i, c], xsem.at[i])
        def w1copy(n):
            return pltpu.make_async_copy(w1_hbm.at[:, cs(n)], w1b.at[n], wsem.at[n])
        def w2copy(n):
            return pltpu.make_async_copy(w2_hbm.at[:, cs(n)], w2b.at[n], wsem.at[8 + n])
        def dwcopy():
            return pltpu.make_async_copy(dw_hbm, dwb, wsem.at[12])
        def ocopy(i, a, n, c):
            return pltpu.make_async_copy(ob.at[i, c, pl.ds(a, n)], o_hbm.at[pl.ds(i * M + (a - m - SH), n), cs(c)], osem.at[0])

        w1copy(CG).start()
        for c in range(CG): xcopy(0, c).start()
        w1copy(0).start()
        dwcopy().start()
        for c in range(1, CG):
            w1copy(CG + c).start(); w1copy(c).start()
        for c in range(CG): w2copy(c).start()

        xb32, w1b32, w2b32 = [r.bitcast(u32) for r in (xb, w1b, w2b)]
        ldx = lambda i, k, r, n: pltpu.bitcast(xb32[i, k, pl.ds(r // 2, n // 2), :], bf16)
        ldw1 = lambda n: pltpu.bitcast(w1b32[n], bf16)
        ldw2 = lambda n: pltpu.bitcast(w2b32[n], bf16)

        def delay(prev, cur, d):
            io = lax.broadcasted_iota(jnp.int32, cur.shape, 1)
            return pltpu.roll(jnp.where(io >= 8 - d, prev, cur), d, 1)

        def shifted(first, cur):
            return first if cur.shape[0] == 1 else jnp.concatenate([first, cur[:-1]], axis=0)

        def conv(c, H, st):
            v = lambda d: dwf[c * K + (K - d)][None]
            Hp = shifted(st[0], H)
            G = delay(Hp, H, 1)
            Gp = shifted(st[1], G)
            n = H.shape[0]
            new = [H[n - 1:], G[n - 1:]]
            Y = (v(8) * Hp + v(9) * Gp) + v(1) * G
            for q, b in enumerate((2, 4, 6)):
                P = ((v(8 + b) * Hp + v(9 + b) * Gp) + v(b) * H) + v(b + 1) * G
                Y = Y + delay(shifted(st[2 + q], P), P, b)
                new.append(P[n - 1:])
            return Y, new

        def act(Y):
            return Y * jnp.tanh(Y) + Y

        def a_ops(i, u, state, flag):
            ops = []
            st = {}
            for c in range(CG):
                def gate(c=c):
                    xv = jnp.concatenate([ldx(i, k, u * m, m) for k in range(CG)], axis=1)
                    b = jnp.dot(xv, ldw1(CG + c), preferred_element_type=f32)
                    st[c] = jnp.tanh(b * 0.5)
                def val(c=c):
                    xv = jnp.concatenate([ldx(i, k, u * m, m) for k in range(CG)], axis=1)
                    a = jnp.dot(xv, ldw1(c), preferred_element_type=f32)
                    H = (a * st[c] + a).reshape(m // 8, 8, 128)
                    if state[c] is None:
                        state[c] = [stb[c * NS + j][None] for j in range(NS)]
                    ys = []
                    j = 0
                    if flag is not None:
                        y, _ = conv(c, jnp.where(flag, 0.0, H[0:1]), state[c])
                        _, state[c] = conv(c, H[0:1], [jnp.where(flag, 0.0, s) for s in state[c]])
                        ys.append(y)
                        j = 1
                    while j < m // 8:
                        e = min(m // 8, (j // (RB // 8) + 1) * (RB // 8))
                        y, state[c] = conv(c, H[j:e], state[c])
                        ys.append(y)
                        j = e
                    Y = jnp.concatenate(ys, axis=0) if len(ys) > 1 else ys[0]
                    sb[c, u * m:(u + 1) * m, :] = act(Y).reshape(m, 128).astype(bf16)
                    if u == U - 1:
                        for j in range(NS):
                            stb[c * NS + j] = state[c][j][0]
                ops += [gate, val]
            return ops

        def c_ops(i, u, n=m):
            ops = []
            p = ((u - 1) % U) * m
            for c in range(CG):
                def op(c=c):
                    sv = jnp.concatenate([sb[k, p:p + n, :] for k in range(CG)], axis=1)
                    o = jnp.dot(sv, ldw2(c), preferred_element_type=f32)
                    ob[i, c, pl.ds(u * m, n), :] = o.astype(bf16)
                ops.append(op)
            return ops

        def run(a, c):
            if order == 0:
                seq = a + c
            elif order == 1:
                seq = []
                for i in range(CG): seq += a[2 * i:2 * i + 2] + c[i:i + 1]
            elif order == 2:
                seq = a[0:2]
                for i in range(CG): seq += a[2 * i + 2:2 * i + 4] + c[i:i + 1]
            elif order == 3:
                seq = []
                for i in range(CG): seq += a[2 * i:2 * i + 1] + c[i:i + 1] + a[2 * i + 1:2 * i + 2]
            for op in seq: op()

        dwcopy().wait()
        dv = dwb[...].astype(f32) * 0.25
        for c in range(CG):
            for k in range(K):
                dwf[c * K + k] = jnp.broadcast_to(dv[k:k + 1, c * 128:(c + 1) * 128], (8, 128))
        for c in range(CG): xcopy(0, c).wait()
        for c in range(2 * CG): w1copy(c).wait()
        for c in range(CG): w2copy(c).wait()
        for c in range(CG): xcopy(1, c).start()
        state = [[jnp.zeros((1, 8, 128), f32)] * NS for _ in range(CG)]
        for u in range(U):
            run(a_ops(0, u, state, None), c_ops(0, u) if u >= 1 else [])
        for c in range(CG): ocopy(0, m + SH, M - m - SH, c).start()

        def body(i, _):
            for c in range(CG): xcopy(i, c).wait()
            @pl.when(i + 1 < N)
            def _():
                for c in range(CG): xcopy(i + 1, c).start()
            fl = i == N // 2
            state = [None] * CG
            for u in range(U):
                run(a_ops(i, u, state, fl if u == 0 else None), c_ops(i, u))
            for c in range(CG): ocopy(i, 0, M, c).start()
            return 0
        lax.fori_loop(1, N, body, 0)

        for c in range(CG):
            y, _ = conv(c, jnp.zeros((1, 8, 128), f32), [stb[c * NS + j][None] for j in range(NS)])
            y = act(y)[0]
            sb[c, M:M + 16, :] = jnp.concatenate([y, y], axis=0).astype(bf16)
        for op in c_ops(N, 0, m + 16): op()
        for c in range(CG): ocopy(N, 0, m + SH, c).start()
        pltpu.make_async_copy(ob.at[pl.ds(0, N)], ob.at[pl.ds(0, N)], osem.at[0]).wait()

    @jax.jit
    def f(x, w1, dw, w2):
        any_ = pl.BlockSpec(memory_space=pl.ANY)
        o = pl.pallas_call(
            kern,
            in_specs=[any_] * 4,
            out_specs=any_,
            out_shape=jax.ShapeDtypeStruct((R, D), bf16),
            scratch_shapes=[
                pltpu.VMEM((N, CG, M, 128), bf16),
                pltpu.VMEM((2 * CG, D, 128), bf16),
                pltpu.VMEM((CG, D, 128), bf16),
                pltpu.VMEM((K, D), bf16),
                pltpu.VMEM((CG * K, 8, 128), f32),
                pltpu.VMEM((CG * NS, 8, 128), f32),
                pltpu.VMEM((CG, M + 16, 128), bf16),
                pltpu.VMEM((N + 1, CG, M, 128), bf16),
                pltpu.SemaphoreType.DMA((N,)),
                pltpu.SemaphoreType.DMA((13,)),
                pltpu.SemaphoreType.DMA((1,)),
            ],
            compiler_params=pltpu.CompilerParams(vmem_limit_bytes=100 * 1024 * 1024, flags=flags, disable_bounds_checks=nbc),
            name="v6",
        )(x.reshape(R, D), w1, dw, w2)
        return o.reshape(B, T, D)
    return f


@jax.jit
def pallas_standalone__conformer_conv_module__speech_kernel(x, w_pw1, dw, w_pw2):
    return make(m=80, U=10, nbc=True)(x, w_pw1, dw, w_pw2)
```

```python
import jax
import jax.numpy as jnp
import numpy as np
from jax import lax
import jax.experimental.pallas as pl
import jax.experimental.pallas.tpu as pltpu

_B, _T, _D, _K = 2, 4000, 512, 15
_R = _B * _T
_G = _D // 128

_LAG = 8

_HEAD0_X = 496
_HEAD0 = _HEAD0_X - 16
_HEAD1_BLOCKS = (112, 112)
_HEAD1 = sum(_HEAD1_BLOCKS)
_HEAD = _HEAD0 + _HEAD1

_BLOCK = 96
_NBLOCK = 19
_CHUNK = _BLOCK * _NBLOCK
_NCHUNK = 4
_DEFER = (1, 5, 10, 15)
_WRITE_BACK = (7, 11, 13, 14, 15, 16, 17, 18)

_SEAM_CHUNK, _SEAM_ROW = divmod(_T - _HEAD - _LAG, _CHUNK)

assert _HEAD + _NCHUNK * _CHUNK == _R
assert _SEAM_CHUNK >= 0 and _SEAM_ROW < _CHUNK - _BLOCK and _SEAM_ROW % 8 == 0

_VAL, _GATE, _OUT, _SPARE = 0, _G * _D, 2 * _G * _D, 3 * _G * _D
_PIN_ROW = _HEAD0_X - 208

_SEM_DW, _SEM_X1, _SEM_W2, _SEM_X, _SEM_OUT, _SEM_HEAD = range(6)

_NEG_LOG2E = np.float32(-np.log2(np.e))


def _sigmoid(v):
    return pltpu.reciprocal(1.0 + jnp.exp2(v * _NEG_LOG2E), approx=True)


def _lanes(g):
    return pl.ds(g * 128, 128)


def _load(ref, row, n):
    words = ref.at[pl.ds(row, n)].bitcast(jnp.uint32)[...]
    return pltpu.bitcast(words, jnp.bfloat16)


def _previous(first, cur):
    return first if cur.shape[0] == 1 else jnp.concatenate([first, cur[:-1]], axis=0)


def _delay(prev, cur, d):
    row = lax.broadcasted_iota(jnp.int32, cur.shape, 1)
    return pltpu.roll(jnp.where(row >= 8 - d, prev, cur), d, 1)


def _filter(taps, h, state):
    w = lambda d: taps[_K - d][None]
    n = h.shape[0]
    h8 = _previous(state[0], h)
    h1 = _delay(h8, h, 1)
    h9 = _previous(state[1], h1)
    new_state = [h[n - 1:], h1[n - 1:]]
    y = (w(8) * h8 + w(9) * h9) + w(1) * h1
    for i, b in enumerate((2, 4, 6)):
        part = ((w(8 + b) * h8 + w(9 + b) * h9) + w(b) * h) + w(b + 1) * h1
        y = y + _delay(_previous(state[2 + i], part), part, b)
        new_state.append(part[n - 1:])
    return y, new_state


def _kernel(x_hbm, w1_hbm, dw_hbm, w2_hbm, o_hbm,
            w_buf, x00, x01, x02, x03, x1_buf, x_buf, o_head, o_buf, dw_buf, tail, sem):
    f32, bf16 = jnp.float32, jnp.bfloat16
    x0_bufs = [x00, x01, x02, x03]
    empty = [jnp.zeros((1, 8, 128), f32)] * 5

    def copy(src, dst, s):
        return pltpu.make_async_copy(src, dst, sem.at[s])

    def start(copies):
        for c in copies:
            c.start()

    def wait(copies):
        for c in copies:
            c.wait()

    def fetch_x(row, n, dst, s):
        return [copy(x_hbm.at[pl.ds(row, n), _lanes(g)], dst(g), s) for g in range(_G)]

    def fetch_chunk(i):
        n = _CHUNK - _LAG
        end = jnp.minimum(_HEAD + (i + 1) * _CHUNK, _R - _LAG)
        return (fetch_x(_HEAD + _LAG + i * _CHUNK, n,
                        lambda g: x_buf.at[i, g, pl.ds(0, n)], _SEM_X)
                + fetch_x(end, _LAG, lambda g: x_buf.at[i, g, pl.ds(n, _LAG)], _SEM_X))

    def write_back(src, lo, hi, row0, g):
        copy(src.at[g, pl.ds(lo, hi - lo)],
             o_hbm.at[pl.ds(row0 + lo, hi - lo), _lanes(g)], _SEM_OUT).start()

    def matmul(lhs, base, g):
        return jnp.dot(jnp.concatenate(lhs, axis=1), _load(w_buf, base + g * _D, _D),
                       preferred_element_type=f32)

    def activate(y):
        return (y * _sigmoid(y)).reshape(y.shape[0] * 8, 128).astype(bf16)

    def front(state, xs, row, n, seam=None, is_end=None, save_tail=False):
        acts, vals = [], []
        for g in range(_G):
            gate = _sigmoid(matmul([_load(x, row, n) for x in xs], _GATE, g))
            vals.append(matmul([_load(x, row, n) for x in xs], _VAL, g))
            h = (vals[g] * gate).reshape(n // 8, 8, 128)
            if is_end is not None:
                h = jnp.concatenate([h[:-1], jnp.where(is_end, 0.0, h[-1:])], axis=0)
            ys, j = [], 0
            if seam is not None:
                j, is_seam = seam
                if j:
                    y, state[g] = _filter(taps[g], h[:j], state[g])
                    ys.append(y)
                ys.append(_filter(taps[g], jnp.where(is_seam, 0.0, h[j:j + 1]), state[g])[0])
                cleared = [jnp.where(is_seam, 0.0, s) for s in state[g]]
                state[g] = _filter(taps[g], h[j:j + 1], cleared)[1]
                j += 1
            if j < h.shape[0]:
                y, state[g] = _filter(taps[g], h[j:], state[g])
                ys.append(y)
            if save_tail:
                tail[2 * g:2 * g + 2] = h[-2:]
            acts.append(activate(jnp.concatenate(ys, axis=0) if len(ys) > 1 else ys[0]))
        return acts, vals

    def back(dst, row, acts, g):
        dst[g, pl.ds(row, acts[0].shape[0]), :] = matmul(acts, _OUT, g).astype(bf16)

    arrivals = []
    for k in range(_G):
        s = _SEM_HEAD + _G + k
        arrivals.append(
            [copy(x_hbm.at[pl.ds(0, _HEAD0_X), _lanes(k)], x0_bufs[k], s)]
            + [copy(w1_hbm.at[_lanes(k), _lanes(_G + g)],
                    w_buf.at[pl.ds(_GATE + g * _D + k * 128, 128)], s) for g in range(_G)])
    for g in range(_G):
        arrivals.append([copy(w1_hbm.at[:, _lanes(g)],
                              w_buf.at[pl.ds(_VAL + g * _D, _D)], _SEM_HEAD + g)])
    arrivals.append(fetch_x(_HEAD0 + _LAG, _HEAD1,
                            lambda g: x1_buf.at[g, pl.ds(0, _HEAD1)], _SEM_X1))
    fetch_w2 = [copy(w2_hbm.at[:, _lanes(g)], w_buf.at[pl.ds(_OUT + g * _D, _D)], _SEM_W2)
                for g in range(_G)]
    fetch_dw = [copy(dw_hbm, dw_buf, _SEM_DW)]
    deferred = [sum(arrivals[5:8], []), arrivals[8], fetch_w2, fetch_chunk(0)]

    def await_next(step, product):
        parked = product[_PIN_ROW:_PIN_ROW + 16, 0:128].astype(bf16)
        if step + 1 < 2 * _G:
            w_buf[pl.ds(_SPARE + 16 * step, 16), :] = parked
        else:
            x1_buf[0, pl.ds(_HEAD1, 16), :] = parked
        wait(arrivals[step + 1])
        if step < len(deferred):
            start(deferred[step])

    start(arrivals[0] + arrivals[1] + fetch_dw + sum(arrivals[2:5], []))
    wait(arrivals[0])
    gates = None
    for k in range(_G):
        rhs = jnp.concatenate(
            [_load(w_buf, _GATE + g * _D + k * 128, 128) for g in range(_G)], axis=1)
        part = jnp.dot(_load(x0_bufs[k], 0, _HEAD0_X), rhs, preferred_element_type=f32)
        gates = part if gates is None else gates + part
        await_next(k, part)
        if k == 1:
            wait(fetch_dw)
    dw = dw_buf[...].astype(f32)
    taps = [[jnp.broadcast_to(dw[k:k + 1, g * 128:(g + 1) * 128], (8, 128))
             for k in range(_K)] for g in range(_G)]
    gates = _sigmoid(gates)
    state, acts = [], []
    for g in range(_G):
        val = matmul([_load(x, 0, _HEAD0_X) for x in x0_bufs], _VAL, g)
        await_next(_G + g, val)
        h = (val * gates[:, g * 128:(g + 1) * 128]).reshape(_HEAD0_X // 8, 8, 128)
        y, st = _filter(taps[g], h[:-1], empty)
        state.append(st)
        acts.append(activate(y[1:]))

    pending = [(r, [a[r:r + _BLOCK] for a in acts]) for r in range(0, _HEAD0, _BLOCK)]
    row = 0
    for u, n in enumerate(_HEAD1_BLOCKS):
        acts, vals = front(state, [x1_buf.at[k] for k in range(_G)], row, n,
                           save_tail=u == len(_HEAD1_BLOCKS) - 1)
        pending.append((_HEAD0 + row, acts))
        row += n
    w_buf[pl.ds(_SPARE + 16 * 2 * _G, 16), :] = vals[2][0:16].astype(bf16)
    wait(fetch_w2)
    for u, block in enumerate(pending):
        for g in range(_G):
            back(o_head, *block, g)
            if u == len(pending) - 1:
                write_back(o_head, 0, _HEAD, 0, g)

    def chunk(i, carry):
        wait(fetch_chunk(i))

        @pl.when(i + 1 < _NCHUNK)
        def _():
            start(fetch_chunk(i + 1))

        xs = [x_buf.at[i, k] for k in range(_G)]
        dst, row0 = o_buf.at[i], _HEAD + i * _CHUNK
        state = [_filter(taps[g], tail[2 * g:2 * g + 2], empty)[1] for g in range(_G)]
        is_seam, is_end = i == _SEAM_CHUNK, i == _NCHUNK - 1
        pending, sent = [], 0
        for u in range(_NBLOCK):
            last = u == _NBLOCK - 1
            seam = (_SEAM_ROW % _BLOCK // 8, is_seam) if u == _SEAM_ROW // _BLOCK else None
            acts, _ = front(state, xs, u * _BLOCK, _BLOCK, seam=seam,
                            is_end=is_end if last else None, save_tail=last)
            ready = len(pending) if last else 0 if u in _DEFER else 1
            for r, a in pending[:ready]:
                for g in range(_G):
                    back(dst, r, a, g)
                if r // _BLOCK + 1 in _WRITE_BACK:
                    for g in range(_G):
                        write_back(dst, sent, r + _BLOCK, row0, g)
                    sent = r + _BLOCK
            pending = pending[ready:] + [(u * _BLOCK, acts)]
        for g in range(_G):
            back(dst, *pending[0], g)
            write_back(dst, sent, _CHUNK, row0, g)
        return carry

    lax.fori_loop(0, _NCHUNK, chunk, 0)
    copy(o_hbm, o_hbm, _SEM_OUT).wait()


@jax.jit
def pallas_standalone__conformer_conv_module__speech_kernel(
    x: jax.Array,
    w_pw1: jax.Array,
    dw: jax.Array,
    w_pw2: jax.Array,
):
    assert x.shape == (_B, _T, _D) and dw.shape == (_K, _D)
    assert w_pw1.shape == (_D, 2 * _D) and w_pw2.shape == (_D, _D)
    bf16 = jnp.bfloat16
    hbm = pl.BlockSpec(memory_space=pl.ANY)
    out = pl.pallas_call(
        _kernel,
        in_specs=[hbm] * 4,
        out_specs=hbm,
        out_shape=jax.ShapeDtypeStruct((_R, _D), bf16),
        scratch_shapes=[
            pltpu.VMEM((_SPARE + 3 * _G * 16, 128), bf16),
            *[pltpu.VMEM((_HEAD0_X, 128), bf16)] * _G,
            pltpu.VMEM((_G, _HEAD1 + 16, 128), bf16),
            pltpu.VMEM((_NCHUNK, _G, _CHUNK, 128), bf16),
            pltpu.VMEM((_G, _HEAD, 128), bf16),
            pltpu.VMEM((_NCHUNK, _G, _CHUNK, 128), bf16),
            pltpu.VMEM((_K, _D), bf16),
            pltpu.VMEM((2 * _G, 8, 128), jnp.float32),
            pltpu.SemaphoreType.DMA((_SEM_HEAD + 2 * _G,)),
        ],
        compiler_params=pltpu.CompilerParams(
            vmem_limit_bytes=64 * 1024 * 1024,
            flags={"XLA_TPU_RESCHEDULE_DMA_DONES": True},
            disable_bounds_checks=True,
        ),
        name="conformer_conv_module",
    )(x.reshape(_R, _D), w_pw1, dw, w_pw2)
    return out.reshape(_B, _T, _D)
```

```python
import jax
import jax.numpy as jnp
import numpy as np
from jax import lax
import jax.experimental.pallas as pl
import jax.experimental.pallas.tpu as pltpu

_B, _T, _D, _K = 2, 4000, 512, 15
_R = _B * _T
_G = _D // 128

_LAG = 8

_HEAD0_X = 496
_HEAD0 = _HEAD0_X - 16
_HEAD0_BLOCK = 96
_HEAD1_BLOCKS = (112, 112)
_HEAD1 = sum(_HEAD1_BLOCKS)
_HEAD = _HEAD0 + _HEAD1

_BLOCKS = (128,) * 12 + (144,) * 2
_CHUNK = sum(_BLOCKS)
_NCHUNK = 4
_DEFER = (1, 5, 9, 12)
_WRITE_BACK = tuple(sum(_BLOCKS[:u]) for u in (5, 8, 10, 11, 12, 13))

_SEAM_CHUNK, _SEAM_ROW = divmod(_T - _HEAD - _LAG, _CHUNK)

assert _HEAD + _NCHUNK * _CHUNK == _R
assert _SEAM_CHUNK >= 0 and _SEAM_ROW < _CHUNK - _BLOCKS[-1] and _SEAM_ROW % 8 == 0

_VAL, _GATE, _OUT, _SPARE = 0, _G * _D, 2 * _G * _D, 3 * _G * _D
_PIN_ROW = _HEAD0_X - 208

_SEM_DW, _SEM_X1, _SEM_W2, _SEM_X, _SEM_OUT, _SEM_HEAD = range(6)

_NEG_LOG2E = np.float32(-np.log2(np.e))


def _sigmoid(v):
    return pltpu.reciprocal(1.0 + jnp.exp2(v * _NEG_LOG2E), approx=True)


def _lanes(g):
    return pl.ds(g * 128, 128)


def _load(ref, row, n):
    return ref[pl.ds(row, n), :]


def _previous(first, cur):
    return first if cur.shape[0] == 1 else jnp.concatenate([first, cur[:-1]], axis=0)


def _delay(prev, cur, d):
    row = lax.broadcasted_iota(jnp.int32, cur.shape, 1)
    return pltpu.roll(jnp.where(row >= 8 - d, prev, cur), d, 1)


def _filter(taps, h, state):
    w = lambda d: taps[_K - d][None]
    n = h.shape[0]
    h8 = _previous(state[0], h)
    h1 = _delay(h8, h, 1)
    h9 = _previous(state[1], h1)
    new_state = [h[n - 1:], h1[n - 1:]]
    y = (w(8) * h8 + w(9) * h9) + w(1) * h1
    for i, b in enumerate((2, 4, 6)):
        part = ((w(8 + b) * h8 + w(9 + b) * h9) + w(b) * h) + w(b + 1) * h1
        y = y + _delay(_previous(state[2 + i], part), part, b)
        new_state.append(part[n - 1:])
    return y, new_state


def _kernel(x_hbm, w1_hbm, dw_hbm, w2_hbm, o_hbm,
            w_buf, x00, x01, x02, x03, x1_buf, x_buf, o_head, o_buf, dw_buf, tail, sem):
    f32, bf16 = jnp.float32, jnp.bfloat16
    x0_bufs = [x00, x01, x02, x03]
    empty = [jnp.zeros((1, 8, 128), f32)] * 5

    def copy(src, dst, s):
        return pltpu.make_async_copy(src, dst, sem.at[s])

    def start(copies):
        for c in copies:
            c.start()

    def wait(copies):
        for c in copies:
            c.wait()

    def fetch_x(row, n, dst, s):
        return [copy(x_hbm.at[pl.ds(row, n), _lanes(g)], dst(g), s) for g in range(_G)]

    def fetch_chunk(i):
        n = _CHUNK - _LAG
        end = jnp.minimum(_HEAD + (i + 1) * _CHUNK, _R - _LAG)
        return (fetch_x(_HEAD + _LAG + i * _CHUNK, n,
                        lambda g: x_buf.at[i, g, pl.ds(0, n)], _SEM_X)
                + fetch_x(end, _LAG, lambda g: x_buf.at[i, g, pl.ds(n, _LAG)], _SEM_X))

    def write_back(src, lo, hi, row0, g):
        copy(src.at[g, pl.ds(lo, hi - lo)],
             o_hbm.at[pl.ds(row0 + lo, hi - lo), _lanes(g)], _SEM_OUT).start()

    def matmul(lhs, base, g):
        return jnp.dot(jnp.concatenate(lhs, axis=1), _load(w_buf, base + g * _D, _D),
                       preferred_element_type=f32)

    def activate(y):
        return (y * _sigmoid(y)).reshape(y.shape[0] * 8, 128).astype(bf16)

    def front(state, xs, row, n, seam=None, is_end=None, save_tail=False):
        acts, vals = [], []
        for g in range(_G):
            gate = _sigmoid(matmul([_load(x, row, n) for x in xs], _GATE, g))
            vals.append(matmul([_load(x, row, n) for x in xs], _VAL, g))
            h = (vals[g] * gate).reshape(n // 8, 8, 128)
            if is_end is not None:
                h = jnp.concatenate([h[:-1], jnp.where(is_end, 0.0, h[-1:])], axis=0)
            ys, j = [], 0
            if seam is not None:
                j, is_seam = seam
                if j:
                    y, state[g] = _filter(taps[g], h[:j], state[g])
                    ys.append(y)
                ys.append(_filter(taps[g], jnp.where(is_seam, 0.0, h[j:j + 1]), state[g])[0])
                cleared = [jnp.where(is_seam, 0.0, s) for s in state[g]]
                state[g] = _filter(taps[g], h[j:j + 1], cleared)[1]
                j += 1
            if j < h.shape[0]:
                y, state[g] = _filter(taps[g], h[j:], state[g])
                ys.append(y)
            if save_tail:
                tail[2 * g:2 * g + 2] = h[-2:]
            acts.append(activate(jnp.concatenate(ys, axis=0) if len(ys) > 1 else ys[0]))
        return acts, vals

    def back(dst, row, acts, g):
        dst[g, pl.ds(row, acts[0].shape[0]), :] = matmul(acts, _OUT, g).astype(bf16)

    arrivals = []
    for k in range(_G):
        s = _SEM_HEAD + _G + k
        arrivals.append(
            [copy(x_hbm.at[pl.ds(0, _HEAD0_X), _lanes(k)], x0_bufs[k], s)]
            + [copy(w1_hbm.at[_lanes(k), _lanes(_G + g)],
                    w_buf.at[pl.ds(_GATE + g * _D + k * 128, 128)], s) for g in range(_G)])
    for g in range(_G):
        arrivals.append([copy(w1_hbm.at[:, _lanes(g)],
                              w_buf.at[pl.ds(_VAL + g * _D, _D)], _SEM_HEAD + g)])
    arrivals.append(fetch_x(_HEAD0 + _LAG, _HEAD1,
                            lambda g: x1_buf.at[g, pl.ds(0, _HEAD1)], _SEM_X1))
    fetch_w2 = [copy(w2_hbm.at[:, _lanes(g)], w_buf.at[pl.ds(_OUT + g * _D, _D)], _SEM_W2)
                for g in range(_G)]
    fetch_dw = [copy(dw_hbm, dw_buf, _SEM_DW)]
    deferred = [sum(arrivals[5:8], []), arrivals[8], fetch_w2, fetch_chunk(0)]

    def await_next(step, product):
        parked = product[_PIN_ROW:_PIN_ROW + 16, 0:128].astype(bf16)
        if step + 1 < 2 * _G:
            w_buf[pl.ds(_SPARE + 16 * step, 16), :] = parked
        else:
            x1_buf[0, pl.ds(_HEAD1, 16), :] = parked
        wait(arrivals[step + 1])
        if step < len(deferred):
            start(deferred[step])

    start(arrivals[0] + arrivals[1] + fetch_dw + sum(arrivals[2:5], []))
    wait(arrivals[0])
    gates = None
    for k in range(_G):
        rhs = jnp.concatenate(
            [_load(w_buf, _GATE + g * _D + k * 128, 128) for g in range(_G)], axis=1)
        part = jnp.dot(_load(x0_bufs[k], 0, _HEAD0_X), rhs, preferred_element_type=f32)
        gates = part if gates is None else gates + part
        await_next(k, part)
        if k == 1:
            wait(fetch_dw)
    dw = dw_buf[...].astype(f32)
    taps = [[jnp.broadcast_to(dw[k:k + 1, g * 128:(g + 1) * 128], (8, 128))
             for k in range(_K)] for g in range(_G)]
    gates = _sigmoid(gates)
    state, acts = [], []
    for g in range(_G):
        val = matmul([_load(x, 0, _HEAD0_X) for x in x0_bufs], _VAL, g)
        await_next(_G + g, val)
        h = (val * gates[:, g * 128:(g + 1) * 128]).reshape(_HEAD0_X // 8, 8, 128)
        y, st = _filter(taps[g], h[:-1], empty)
        state.append(st)
        acts.append(activate(y[1:]))

    pending = [(r, [a[r:r + _HEAD0_BLOCK] for a in acts])
               for r in range(0, _HEAD0, _HEAD0_BLOCK)]
    row = 0
    for u, n in enumerate(_HEAD1_BLOCKS):
        acts, vals = front(state, [x1_buf.at[k] for k in range(_G)], row, n,
                           save_tail=u == len(_HEAD1_BLOCKS) - 1)
        pending.append((_HEAD0 + row, acts))
        row += n
    w_buf[pl.ds(_SPARE + 16 * 2 * _G, 16), :] = vals[2][0:16].astype(bf16)
    wait(fetch_w2)
    for u, block in enumerate(pending):
        for g in range(_G):
            back(o_head, *block, g)
            if u == len(pending) - 1:
                write_back(o_head, 0, _HEAD, 0, g)

    def chunk(i, carry):
        wait(fetch_chunk(i))

        @pl.when(i + 1 < _NCHUNK)
        def _():
            start(fetch_chunk(i + 1))

        xs = [x_buf.at[i, k] for k in range(_G)]
        dst, row0 = o_buf.at[i], _HEAD + i * _CHUNK
        state = [_filter(taps[g], tail[2 * g:2 * g + 2], empty)[1] for g in range(_G)]
        is_seam, is_end = i == _SEAM_CHUNK, i == _NCHUNK - 1
        pending, sent, row = [], 0, 0
        for u, n in enumerate(_BLOCKS):
            last = u == len(_BLOCKS) - 1
            seam = ((_SEAM_ROW - row) // 8, is_seam) if row <= _SEAM_ROW < row + n else None
            acts, _ = front(state, xs, row, n, seam=seam,
                            is_end=is_end if last else None, save_tail=last)
            ready = len(pending) if last else 0 if u in _DEFER else 1
            for r, a in pending[:ready]:
                for g in range(_G):
                    back(dst, r, a, g)
                done = r + a[0].shape[0]
                if done in _WRITE_BACK:
                    for g in range(_G):
                        write_back(dst, sent, done, row0, g)
                    sent = done
            pending = pending[ready:] + [(row, acts)]
            row += n
        for g in range(_G):
            back(dst, *pending[0], g)
            write_back(dst, sent, _CHUNK, row0, g)
        return carry

    lax.fori_loop(0, _NCHUNK, chunk, 0)
    copy(o_hbm, o_hbm, _SEM_OUT).wait()


@jax.jit
def pallas_standalone__conformer_conv_module__speech_kernel(
    x: jax.Array,
    w_pw1: jax.Array,
    dw: jax.Array,
    w_pw2: jax.Array,
):
    assert x.shape == (_B, _T, _D) and dw.shape == (_K, _D)
    assert w_pw1.shape == (_D, 2 * _D) and w_pw2.shape == (_D, _D)
    bf16 = jnp.bfloat16
    hbm = pl.BlockSpec(memory_space=pl.ANY)
    out = pl.pallas_call(
        _kernel,
        in_specs=[hbm] * 4,
        out_specs=hbm,
        out_shape=jax.ShapeDtypeStruct((_R, _D), bf16),
        scratch_shapes=[
            pltpu.VMEM((_SPARE + 3 * _G * 16, 128), bf16),
            *[pltpu.VMEM((_HEAD0_X, 128), bf16)] * _G,
            pltpu.VMEM((_G, _HEAD1 + 16, 128), bf16),
            pltpu.VMEM((_NCHUNK, _G, _CHUNK, 128), bf16),
            pltpu.VMEM((_G, _HEAD, 128), bf16),
            pltpu.VMEM((_NCHUNK, _G, _CHUNK, 128), bf16),
            pltpu.VMEM((_K, _D), bf16),
            pltpu.VMEM((2 * _G, 8, 128), jnp.float32),
            pltpu.SemaphoreType.DMA((_SEM_HEAD + 2 * _G,)),
        ],
        compiler_params=pltpu.CompilerParams(
            vmem_limit_bytes=64 * 1024 * 1024,
            flags={"XLA_TPU_RESCHEDULE_DMA_DONES": True},
            disable_bounds_checks=True,
            disable_semaphore_checks=True,
        ),
        name="conformer_conv_module",
    )(x.reshape(_R, _D), w_pw1, dw, w_pw2)
    return out.reshape(_B, _T, _D)
```
